```python
import jax
import jax.numpy as jnp

def _softmax(x, axis=-1):
    return jax.nn.softmax(x, axis=axis)
def _gelu(x):
    return jax.nn.gelu(x, approximate=True)
def _silu(x):
    return jax.nn.silu(x)
def _sigmoid(x):
    return jax.nn.sigmoid(x)
def _layernorm(x, axis=-1, eps=1e-5):
    m = jnp.mean(x, axis=axis, keepdims=True)
    v = jnp.var(x, axis=axis, keepdims=True)
    return (x - m) / jnp.sqrt(v + eps)
def _scatter_add(tgt, idx, src, axis=0):
    return tgt.at[idx].add(src)
def _segment_sum(src, seg, n):
    return jax.ops.segment_sum(src, seg, n)
class _Rng:
    def __init__(self, key):
        self._k = key
    def _next(self):
        self._k, sub = jax.random.split(self._k)
        return sub
    def normal(self, shape):
        return jax.random.normal(self._next(), shape, dtype=jnp.bfloat16)
    def randint(self, lo, hi, shape):
        return jax.random.randint(self._next(), shape, lo, hi, dtype=jnp.int32)
    def uniform(self, shape, lo=0.0, hi=1.0):
        return jax.random.uniform(self._next(), shape, jnp.bfloat16, lo, hi)
    def permutation(self, n):
        return jax.random.permutation(self._next(), n)


kernel_name = 'recurrent_scan__sliding_block_cached__dense_activation_gelu__decode'

def setup_inputs():
    _rng = _Rng(jax.random.key(int.from_bytes(__import__("os").urandom(4), "little")))
    _w = (lambda a: (lambda t: t.astype(jnp.bfloat16) if jnp.issubdtype(t.dtype, jnp.floating) else t)(jnp.asarray(a)))
    def _A_setup():
        B, Sq, D = 2, 1, 576
        Hq, Hkv, Sk, Dh = 32, 16, 32768, 128
        assert Hq % Hkv == 0, (Hq, Hkv)
        return {
            "x": _w((lambda *s: _rng.normal(s) * 0.05)(B, Sq, D)),
            "k_cache": _w((lambda *s: _rng.normal(s) * 0.05)(B, Hkv, Sk, Dh)),
            "v_cache": _w((lambda *s: _rng.normal(s) * 0.05)(B, Hkv, Sk, Dh)),
            "wq": _w((lambda *s: _rng.normal(s) * 0.05)(D, Hq * Dh) * (D ** -0.5)),
            "wo": _w((lambda *s: _rng.normal(s) * 0.05)(Hq * Dh, D) * ((Hq * Dh) ** -0.5)),
        }
    _A_in = _A_setup()

    def _B_setup():
        B, S, D, F = 2, 1, 576, 4608
        return {
            "x": _w((lambda *s: _rng.normal(s) * 0.05)(B, S, D)),
            "w1": _w((lambda *s: _rng.normal(s) * 0.05)(D, F) * (D ** -0.5)),
            "b1": _w((lambda *s: _rng.normal(s) * 0.05)(F) * 0.01),
            "w2": _w((lambda *s: _rng.normal(s) * 0.05)(F, D) * (F ** -0.5)),
            "b2": _w((lambda *s: _rng.normal(s) * 0.05)(D) * 0.01),
        }
    _B_in = _B_setup()

    return {
        "A_x": _A_in["x"],
        "A_k_cache": _A_in["k_cache"],
        "A_v_cache": _A_in["v_cache"],
        "A_wq": _A_in["wq"],
        "A_wo": _A_in["wo"],
        "B_x": _B_in["x"],
        "B_w1": _B_in["w1"],
        "B_b1": _B_in["b1"],
        "B_w2": _B_in["w2"],
        "B_b2": _B_in["b2"],
    }

def reference(A_x, A_k_cache, A_v_cache, A_wq, A_wo, B_x, B_w1, B_b1, B_w2, B_b2):
    def _A_ref(x, k_cache, v_cache, wq, wo):
        B, Sq, D = x.shape
        Hq, Dh = 32, 128
        Hkv, Sk = k_cache.shape[1], k_cache.shape[2]
        W = min(4096, max(256, Sk // 4))
        rep = Hq // Hkv
        q = (lambda x, *d: x.transpose(*d))((x @ wq).reshape(B, Sq, Hq, Dh), 0, 2, 1, 3)
        k = jnp.repeat(k_cache[:, :, Sk - W:, :], rep, axis=1)
        v = jnp.repeat(v_cache[:, :, Sk - W:, :], rep, axis=1)
        scores = jnp.einsum("bhqd,bhkd->bhqk", q, k) * (Dh ** -0.5)
        p = _softmax(scores, axis=-1)
        o = jnp.einsum("bhqk,bhkd->bhqd", p, v)
        return (lambda x, *d: x.transpose(*d))(o, 0, 2, 1, 3).reshape(B, Sq, Hq * Dh) @ wo

    def _B_ref(x, w1, b1, w2, b2):
        h = jnp.einsum("bsd,df->bsf", x, w1) + b1
        h = _gelu(h)
        return jnp.einsum("bsf,fd->bsd", h, w2) + b2

    x = A_x
    xn = _layernorm(x, axis=-1)
    s = _A_ref(xn, A_k_cache, A_v_cache, A_wq, A_wo)
    g = _silu(_B_ref(xn, B_w1, B_b1, B_w2, B_b2))
    return x + s * g
```

```python
import functools
import jax
import jax.numpy as jnp
from jax import lax
import jax.experimental.pallas as pl
import jax.experimental.pallas.tpu as pltpu

HQ, DH = 32, 128
NT = (((1,), (1,)), ((), ()))
F32 = jnp.float32
BF16 = jnp.bfloat16


def _interleave(issues, pieces):
    n, m = len(issues), len(pieces)
    for j, piece in enumerate(pieces):
        for t in range(j * n // m, (j + 1) * n // m):
            issues[t](t % 2)
        piece()


def _kernel(x_hbm, k_hbm, v_hbm, wq_hbm, wot_hbm, w1_hbm, b1_hbm, w2t_hbm, b2_hbm,
            o_ref,
            x_v, b1_v, b2_v, wq_v, wot_v, w1_v, w2t_v, kbuf, vbuf, q_v, h_v, s_v, p_v, oc_v,
            sem_s, sem_w, sem_o, sem_k, sem_v, *, W, CH, RW, CSPLIT, NS, NPIECE):
    B, HKV, SK, _ = k_hbm.shape
    D = x_v.shape[1]
    F = w1_v.shape[1]
    NCH = W // CH

    def w_issues(src, dst, sem, r0, r1, ns):
        cols = src.shape[1]
        cw = cols // CSPLIT
        per = (r1 - r0) // RW // ns
        out = []
        for t in range(per):
            for c in range(CSPLIT):
                for s in range(ns):
                    r = r0 + (s * per + t) * RW
                    sl = (pl.ds(r, RW), pl.ds(c * cw, cw))
                    out.append(lambda pr, sl=sl: pltpu.make_async_copy(src.at[sl], dst.at[sl], sem).start(priority=pr))
        return out

    def kv_issues(h):
        out = []
        for c in range(NCH):
            for b in range(B):
                for src, dst, sem in ((k_hbm, kbuf, sem_k), (v_hbm, vbuf, sem_v)):
                    def f(pr, c=c, b=b, src=src, dst=dst, sem=sem):
                        i = h * B + b
                        pltpu.make_async_copy(src.at[b, h, pl.ds(SK - W + c * CH, CH), :],
                                              dst.at[i, pl.ds(c * CH, CH), :], sem.at[i]).start(priority=pr)
                    out.append(f)
        return out

    def wait_all(ref, sem):
        pltpu.make_async_copy(ref, ref, sem).wait()

    c_x = pltpu.make_async_copy(x_hbm, x_v, sem_s.at[0])
    c_b1 = pltpu.make_async_copy(b1_hbm, b1_v, sem_s.at[1])
    c_b2 = pltpu.make_async_copy(b2_hbm, b2_v, sem_s.at[2])

    st = {}

    def ln():
        c_x.wait()
        xs = x_v[...].astype(F32)
        row = lax.broadcasted_iota(jnp.int32, (8, D), 0)
        x8 = jnp.where(row % 2 == 0, xs[0:1, :], xs[1:2, :])
        m = jnp.mean(x8, axis=-1, keepdims=True)
        xc = x8 - m
        var = jnp.mean(xc * xc, axis=-1, keepdims=True)
        st["xs"] = xs
        st["xn"] = (xc / jnp.sqrt(var + 1e-5)).astype(BF16)

    def small():
        c_x.start()
        c_b1.start()
        c_b2.start()

    nop = lambda: None
    _interleave(w_issues(wq_hbm, wq_v, sem_w.at[0], 0, D, NS), [small, nop, nop, ln])

    def qproj(j, n):
        def f():
            if j == 0:
                wait_all(wq_v, sem_w.at[0])
            cw = HQ * DH // n
            q_v[:, j * cw:(j + 1) * cw] = jnp.dot(st["xn"], wq_v[:, j * cw:(j + 1) * cw], preferred_element_type=F32)
        return f
    _interleave(w_issues(w1_hbm, w1_v, sem_w.at[1], 0, D, NS), [nop] + [qproj(j, 8) for j in range(8)])

    def hproj(j, n):
        def f():
            if j == 0:
                c_b1.wait()
                c_b2.wait()
                wait_all(w1_v, sem_w.at[1])
            nt = F // 128 // n
            for t in range(j * nt, (j + 1) * nt):
                hj = jnp.dot(st["xn"], w1_v[:, t * 128:(t + 1) * 128], preferred_element_type=F32)
                hj = hj + b1_v[t:t + 1, :].astype(F32)
                h_v[:, t * 128:(t + 1) * 128] = jax.nn.gelu(hj, approximate=True)
        return f
    _interleave(w_issues(w2t_hbm, w2t_v, sem_w.at[2], 0, D, NS), [nop] + [hproj(j, 9) for j in range(9)])

    def yproj(j, n):
        def f():
            if j == 0:
                wait_all(w2t_v, sem_w.at[2])
                st["y"] = b2_v[...].astype(F32).reshape(1, D)
            cw = F // n
            st["y"] = st["y"] + lax.dot_general(h_v[:, j * cw:(j + 1) * cw].astype(BF16), w2t_v[:, j * cw:(j + 1) * cw], NT,
                                                preferred_element_type=F32)
        return f
    _interleave(kv_issues(0), [nop] + [yproj(j, 9) for j in range(9)])
    y = st["y"]
    g = y * jax.nn.sigmoid(y)

    scale = DH ** -0.5
    r8 = lax.broadcasted_iota(jnp.int32, (8, DH), 0)

    def head_pieces(h):
        c0 = pl.multiple_of(h * 256, 256)
        hs = {}
        pieces = []
        n = NPIECE
        cw = W // n
        for b in range(B):
            i = h * B + b
            for j in range(n):
                def qk(b=b, i=i, j=j):
                    if b == 0 and j == 0:
                        qa = q_v[:, pl.ds(c0, 128)]
                        qb = q_v[:, pl.ds(c0 + 128, 128)]
                        hs["q"] = jnp.where(r8 < 2, qa, qb).astype(BF16)
                    if j == 0:
                        wait_all(kbuf.at[i], sem_k.at[i])
                    s_v[:, j * cw:(j + 1) * cw] = lax.dot_general(hs["q"], kbuf[i, j * cw:(j + 1) * cw, :], NT,
                                                                  preferred_element_type=F32) * scale
                pieces.append(qk)
            for j in range(n):
                def pv(b=b, i=i, j=j):
                    if j == 0:
                        s = s_v[...]
                        mx = jnp.max(s, axis=-1, keepdims=True)
                        p = jnp.exp(s - mx)
                        hs["l"] = jnp.sum(p, axis=-1, keepdims=True)
                        p_v[...] = p
                        wait_all(vbuf.at[i], sem_v.at[i])
                        hs["o"] = jnp.zeros((8, DH), F32)
                    hs["o"] = hs["o"] + jnp.dot(p_v[:, j * cw:(j + 1) * cw].astype(BF16), vbuf[i, j * cw:(j + 1) * cw, :],
                                                preferred_element_type=F32)
                    if j == n - 1:
                        hs["o%d" % b] = hs["o"] / hs["l"]
                        if b == B - 1:
                            o = jnp.where(r8 % 2 == 0, hs["o0"], hs["o1"])
                            oc_v[:, pl.ds(c0, 128)] = jnp.where(r8 < 2, o, 0.0)
                            oc_v[:, pl.ds(c0 + 128, 128)] = jnp.where((r8 >= 2) & (r8 < 4), o, 0.0)
                pieces.append(pv)
        return pieces

    def body(h, c):
        _interleave(kv_issues(h + 1), head_pieces(h))
        return c
    lax.fori_loop(0, HKV - 1, body, 0)

    groups = [(r, min(r + 128, D)) for r in range(0, D, 128)]
    gi = [w_issues(wot_hbm, wot_v, sem_o.at[t], r0, r1, NS) for t, (r0, r1) in enumerate(groups)]
    _interleave(gi[0] + gi[1], head_pieces(HKV - 1))

    def oproj(t):
        def f():
            r0, r1 = groups[t]
            if t == 0:
                st["oc"] = oc_v[...].astype(BF16)
            wait_all(wot_v.at[pl.ds(r0, r1 - r0), :], sem_o.at[t])
            acc = lax.dot_general(st["oc"], wot_v[r0:r1, :], NT, preferred_element_type=F32)
            s = acc[0:2, :] + acc[2:4, :]
            o_ref[:, r0:r1] = (st["xs"][:, r0:r1] + s * g[0:2, r0:r1]).astype(o_ref.dtype)
        return f
    _interleave(gi[2], [oproj(0)])
    _interleave(gi[3], [oproj(1)])
    _interleave(gi[4], [oproj(2)])
    oproj(3)()
    oproj(4)()


@jax.jit
def pallas_recurrent_scan__sliding_block_cached__dense_activation_gelu__decode_kernel(
    A_x, A_k_cache, A_v_cache, A_wq, A_wo, B_x, B_w1, B_b1, B_w2, B_b2):
    CH, RW, CSPLIT, NS, NPIECE = 128, 8, 2, 4, 1
    B, Sq, D = A_x.shape
    _, HKV, SK, _ = A_k_cache.shape
    F = B_w1.shape[1]
    W = min(4096, max(256, SK // 4))
    bf = jnp.bfloat16
    anyspec = pl.BlockSpec(memory_space=pl.ANY)
    out = pl.pallas_call(
        functools.partial(_kernel, W=W, CH=CH, RW=RW, CSPLIT=CSPLIT, NS=NS, NPIECE=NPIECE),
        out_shape=jax.ShapeDtypeStruct((B, D), A_x.dtype),
        in_specs=[anyspec] * 9,
        out_specs=pl.BlockSpec(memory_space=pltpu.VMEM),
        scratch_shapes=[
            pltpu.VMEM((B, D), bf), pltpu.VMEM((F // 128, 128), bf), pltpu.VMEM((D,), bf),
            pltpu.VMEM((D, HQ * DH), bf), pltpu.VMEM((D, HQ * DH), bf),
            pltpu.VMEM((D, F), bf), pltpu.VMEM((D, F), bf),
            pltpu.VMEM((B * HKV, W, DH), bf), pltpu.VMEM((B * HKV, W, DH), bf),
            pltpu.VMEM((8, HQ * DH), F32), pltpu.VMEM((8, F), F32),
            pltpu.VMEM((8, W), F32), pltpu.VMEM((8, W), F32), pltpu.VMEM((8, HQ * DH), F32),
            pltpu.SemaphoreType.DMA((3,)), pltpu.SemaphoreType.DMA((3,)), pltpu.SemaphoreType.DMA((5,)),
            pltpu.SemaphoreType.DMA((B * HKV,)), pltpu.SemaphoreType.DMA((B * HKV,)),
        ],
        compiler_params=pltpu.CompilerParams(vmem_limit_bytes=110 * 1024 * 1024),
    )(A_x.reshape(B, D), A_k_cache, A_v_cache, A_wq, A_wo.T, B_w1, B_b1.reshape(F // 128, 128), B_w2.T, B_b2)
    return out.reshape(B, Sq, D)
```

```python
import functools
import jax
import jax.numpy as jnp
from jax import lax
import jax.experimental.pallas as pl
import jax.experimental.pallas.tpu as pltpu

HQ, DH = 32, 128
NT = (((1,), (1,)), ((), ()))
F32 = jnp.float32
BF16 = jnp.bfloat16


def _kernel(x_hbm, k_hbm, v_hbm, wq_hbm, wot_hbm, w1_hbm, b1_hbm, w2t_hbm, b2_hbm,
            o_ref,
            x_v, b1_v, b2_v, wq_v, wot_v, w1_v, w2t_v, kv,
            b1f_v, q_v, h_v, s_v, oc_v,
            sem, *, W, CH, G, CS, NQ, PRE, LA, WPRE, NSL):
    B, HKV, SK, _ = k_hbm.shape
    D = x_v.shape[1]
    F = w1_v.shape[1]
    NCH = W // CH
    NP = B * HKV
    PG = B * G
    SPP = NCH // PG
    RW, NS = 8, 4
    SR, RING = 4, 3
    SQ = SR + RING
    assert NSL * PG >= LA
    assert NSL * PG + LA >= 5
    WST = D // RW // NS

    def w_step(src, dst, sem, r0, per, t, cs):
        cw = src.shape[1] // cs
        n = 0
        for c in range(cs):
            for s in range(NS):
                r = pl.multiple_of(r0 + (s * per + t) * RW, RW)
                sl = (pl.ds(r, RW), pl.ds(c * cw, cw))
                pltpu.make_async_copy(src.at[sl], dst.at[sl], sem).start(priority=n % 2)
                n += 1

    def w_steps(src, dst, sem, t0, n, r0=0, per=WST, cs=CS):
        def f(t, c):
            w_step(src, dst, sem, r0, per, t0 + t, cs)
            return c
        lax.fori_loop(0, n, f, 0)

    def kv_steps(s0, n):
        def f(t, c):
            s = s0 + t
            g = lax.div(s, NCH)
            off = pl.multiple_of(lax.rem(s, NCH) * CH, CH)
            for hh in range(G):
                h = g * G + hh
                for b in range(B):
                    i = h * B + b
                    for pr, (src, dst) in enumerate(((k_hbm, kv.at[0]), (v_hbm, kv.at[1]))):
                        pltpu.make_async_copy(src.at[b, h, pl.ds(SK - W + off, CH), :],
                                              dst.at[i, pl.ds(off, CH), :], sem.at[SR + lax.rem(g, RING)]).start(priority=pr)
            return c
        lax.fori_loop(0, n, f, 0)

    def wait_all(ref, sem):
        pltpu.make_async_copy(ref, ref, sem).wait()

    c_x = pltpu.make_async_copy(x_hbm, x_v, sem.at[SQ])
    c_b1 = pltpu.make_async_copy(b1_hbm, b1_v, sem.at[SQ])
    c_b2 = pltpu.make_async_copy(b2_hbm, b2_v, sem.at[SQ])

    c_x.start()
    c_b1.start()
    c_b2.start()
    w_steps(wq_hbm, wq_v, sem.at[0], 0, WST // 2)
    c_x.wait()
    c_b1.wait()
    c_b2.wait()
    xs = x_v[...].astype(F32)
    row = lax.broadcasted_iota(jnp.int32, (8, D), 0)
    x8 = jnp.where(row % 2 == 0, xs[0:1, :], xs[1:2, :])
    m = jnp.mean(x8, axis=-1, keepdims=True)
    xc = x8 - m
    var = jnp.mean(xc * xc, axis=-1, keepdims=True)
    xn = (xc / jnp.sqrt(var + 1e-5)).astype(BF16)
    b1f_v[...] = b1_v[...].astype(F32)
    y0 = jnp.broadcast_to(b2_v[...].astype(F32).reshape(1, D), (8, D))
    w_steps(wq_hbm, wq_v, sem.at[0], WST // 2, WST - WST // 2)

    w_steps(w1_hbm, w1_v, sem.at[1], 0, WPRE)
    nw = (WST - WPRE) // 2
    wait_all(wq_v, sem.at[0])

    def qproj(j, c):
        c0 = pl.multiple_of(j * 512, 512)
        q_v[:, pl.ds(c0, 512)] = jnp.dot(xn, wq_v[:, pl.ds(c0, 512)], preferred_element_type=F32)

        @pl.when(j < nw)
        def _():
            w_steps(w1_hbm, w1_v, sem.at[1], WPRE + 2 * j, 2)
        return c
    lax.fori_loop(0, HQ * DH // 512, qproj, 0)

    w_steps(w2t_hbm, w2t_v, sem.at[2], 0, WPRE)
    wait_all(w1_v, sem.at[1])

    def hproj(j, c):
        c0 = pl.multiple_of(j * 512, 512)
        hj = jnp.dot(xn, w1_v[:, pl.ds(c0, 512)], preferred_element_type=F32)
        bb = b1f_v[pl.ds(j * 4, 4), :]
        hj = hj + jnp.concatenate([bb[t:t + 1, :] for t in range(4)], axis=1)
        h_v[:, pl.ds(c0, 512)] = jax.nn.gelu(hj, approximate=True)

        @pl.when(j < nw)
        def _():
            w_steps(w2t_hbm, w2t_v, sem.at[2], WPRE + 2 * j, 2)
        return c
    lax.fori_loop(0, F // 512, hproj, 0)

    ks = (NCH - PRE) // 8
    kv_steps(0, NCH - 8 * ks)
    wait_all(w2t_v, sem.at[2])

    def yproj(j, y):
        c0 = pl.multiple_of(j * 512, 512)
        y = y + lax.dot_general(h_v[:, pl.ds(c0, 512)].astype(BF16), w2t_v[:, pl.ds(c0, 512)], NT,
                                preferred_element_type=F32)

        @pl.when(j < 8)
        def _():
            kv_steps(NCH - 8 * ks + ks * j, ks)
        return y
    y = lax.fori_loop(0, F // 512, yproj, y0)
    gate = y * jax.nn.sigmoid(y)
    kv_steps(NCH, LA * (SPP // NSL))

    scale = DH ** -0.5
    r8 = lax.broadcasted_iota(jnp.int32, (8, DH), 0)
    RL = 512
    qw = HQ * DH // NQ
    qcs = max(1, CS // NQ) if qw * RW * 2 > 32768 else 1
    SPS = SPP // NSL

    def issue(i, part):
        slot = NSL * (i + PG) + part + LA

        @pl.when(slot < NSL * NP)
        def _():
            kv_steps(slot * SPS, SPS)

        @pl.when(slot >= NSL * NP)
        def _():
            t = slot - NSL * NP

            @pl.when(t < RL // 128)
            def _():
                w_steps(wot_hbm, wot_v, sem.at[t], 0, 4, r0=t * 128, per=4)

            @pl.when(t == RL // 128)
            def _():
                for qi in range(NQ):
                    cw = qw // qcs
                    n = 0
                    for cc in range(qcs):
                        for r in range(RL, D, RW):
                            sl = (pl.ds(r, RW), pl.ds(qi * qw + cc * cw, cw))
                            pltpu.make_async_copy(wot_hbm.at[sl], wot_v.at[sl], sem.at[SQ + qi]).start(priority=n % 2)
                            n += 1

    def pair(i, c):
        h = lax.div(i, B)
        b = lax.rem(i, B)
        c0 = pl.multiple_of(h * 256, 256)
        hw = W // (NSL // 2)
        qh = jnp.where(r8 < 2, q_v[:, pl.ds(c0, 128)], q_v[:, pl.ds(c0 + 128, 128)]).astype(BF16)
        for j in range(NSL // 2):
            issue(i, j)
            if j == 0:
                @pl.when(lax.rem(i, PG) == 0)
                def _():
                    wait_all(kv.at[:, pl.ds(i, PG)], sem.at[SR + lax.rem(lax.div(i, PG), RING)])
            s_v[:, j * hw:(j + 1) * hw] = lax.dot_general(qh, kv[0, i, j * hw:(j + 1) * hw, :], NT,
                                                          preferred_element_type=F32) * scale
        s = s_v[...]
        mx = jnp.max(s, axis=-1, keepdims=True)
        p = jnp.exp(s - mx)
        l = jnp.sum(p, axis=-1, keepdims=True)
        s_v[...] = p
        o = jnp.zeros((8, DH), F32)
        for j in range(NSL // 2):
            issue(i, NSL // 2 + j)
            o = o + jnp.dot(s_v[:, j * hw:(j + 1) * hw].astype(BF16), kv[1, i, j * hw:(j + 1) * hw, :],
                            preferred_element_type=F32)
        o = o / l
        r0 = pl.multiple_of(b * 8, 8)
        oc_v[pl.ds(r0, 8), pl.ds(c0, 128)] = jnp.where(r8 == b, o, 0.0)
        oc_v[pl.ds(r0, 8), pl.ds(c0 + 128, 128)] = jnp.where(r8 == 2 + b, o, 0.0)
        return c
    lax.fori_loop(0, NP, pair, 0)

    oc = oc_v[...].astype(BF16)

    def oproj(t, c):
        r0 = pl.multiple_of(t * 128, 128)
        wait_all(wot_v.at[pl.ds(r0, 128), :], sem.at[t])
        oq = lax.dot_general(oc, wot_v[pl.ds(r0, 128), :], NT, preferred_element_type=F32)
        s_v[:, pl.ds(r0, 128)] = oq[0:8, :] + oq[8:16, :]
        return c
    lax.fori_loop(0, RL // 128, oproj, 0)
    sa = s_v[:, 0:RL]
    o_ref[:, 0:RL] = (xs[:, 0:RL] + (sa[0:2, :] + sa[2:4, :]) * gate[0:2, 0:RL]).astype(o_ref.dtype)
    acc = jnp.zeros((16, D - RL), F32)
    for qi in range(NQ):
        sl = (pl.ds(RL, D - RL), pl.ds(qi * qw, qw))
        wait_all(wot_v.at[sl], sem.at[SQ + qi])
        acc = acc + lax.dot_general(oc[:, qi * qw:(qi + 1) * qw], wot_v[sl], NT, preferred_element_type=F32)
    sb = acc[0:8, :] + acc[8:16, :]
    o_ref[:, RL:D] = (xs[:, RL:D] + (sb[0:2, :] + sb[2:4, :]) * gate[0:2, RL:D]).astype(o_ref.dtype)


@jax.jit
def pallas_recurrent_scan__sliding_block_cached__dense_activation_gelu__decode_kernel(
    A_x, A_k_cache, A_v_cache, A_wq, A_wo, B_x, B_w1, B_b1, B_w2, B_b2):
    CH = 128
    G = 1
    CS = 2
    NQ = 2
    PRE = 16
    LA = 2
    WPRE = 6
    NSL = 2
    B, Sq, D = A_x.shape
    _, HKV, SK, _ = A_k_cache.shape
    F = B_w1.shape[1]
    W = min(4096, max(256, SK // 4))
    bf = jnp.bfloat16
    anyspec = pl.BlockSpec(memory_space=pl.ANY)
    out = pl.pallas_call(
        functools.partial(_kernel, W=W, CH=CH, G=G, CS=CS, NQ=NQ, PRE=PRE, LA=LA, WPRE=WPRE, NSL=NSL),
        out_shape=jax.ShapeDtypeStruct((B, D), A_x.dtype),
        in_specs=[anyspec] * 9,
        out_specs=pl.BlockSpec(memory_space=pltpu.VMEM),
        scratch_shapes=[
            pltpu.VMEM((B, D), bf), pltpu.VMEM((F // 128, 128), bf), pltpu.VMEM((D,), bf),
            pltpu.VMEM((D, HQ * DH), bf), pltpu.VMEM((D, HQ * DH), bf),
            pltpu.VMEM((D, F), bf), pltpu.VMEM((D, F), bf),
            pltpu.VMEM((2, B * HKV, W, DH), bf),
            pltpu.VMEM((F // 128, 128), F32), pltpu.VMEM((8, HQ * DH), F32), pltpu.VMEM((8, F), F32),
            pltpu.VMEM((8, W), F32), pltpu.VMEM((16, HQ * DH), F32),
            pltpu.SemaphoreType.DMA((7 + NQ,)),
        ],
        compiler_params=pltpu.CompilerParams(vmem_limit_bytes=110 * 1024 * 1024, disable_bounds_checks=True),
    )(A_x.reshape(B, D), A_k_cache, A_v_cache, A_wq, A_wo.T, B_w1, B_b1.reshape(F // 128, 128), B_w2.T, B_b2)
    return out.reshape(B, Sq, D)
```

```python
import functools
import jax
import jax.numpy as jnp
from jax import lax
import jax.experimental.pallas as pl
import jax.experimental.pallas.tpu as pltpu

HQ, DH = 32, 128
NT = (((1,), (1,)), ((), ()))
F32 = jnp.float32
BF16 = jnp.bfloat16


def _kernel(x_hbm, k_hbm, v_hbm, wq_hbm, wot_hbm, w1_hbm, b1_hbm, w2t_hbm, b2_hbm,
            o_ref,
            x_v, b1_v, b2_v, wq_v, wot_v, w1_v, w2t_v, kv,
            b1f_v, q_v, h_v, s_v, oc_v,
            sem, *, W, CH, G, CS, NQ, PRE, LA, WPRE, NSL, NS, HS):
    B, HKV, SK, _ = k_hbm.shape
    D = x_v.shape[1]
    F = w1_v.shape[1]
    NCH = W // CH // HS
    NP = B * HKV
    PG = B * G
    SPP = NCH // PG
    RW = 8
    SR, RING = 4, 3
    SQ = SR + RING
    assert NSL * PG >= LA
    assert NSL * PG + LA >= 5
    WS = D // RW // NS // 9
    OS = 128 // RW // NS
    WST = D // RW // NS

    def w_step(src, dst, sem, r0, per, t, cs):
        cw = src.shape[1] // cs
        n = 0
        for c in range(cs):
            for s in range(NS):
                r = pl.multiple_of(r0 + (s * per + t) * RW, RW)
                sl = (pl.ds(r, RW), pl.ds(c * cw, cw))
                pltpu.make_async_copy(src.at[sl], dst.at[sl], sem).start(priority=n % 2)
                n += 1

    def w_steps(src, dst, sem, t0, n, r0=0, per=WST, cs=CS):
        def f(t, c):
            w_step(src, dst, sem, r0, per, t0 + t, cs)
            return c
        lax.fori_loop(0, n, f, 0)

    def kv_steps(s0, n):
        def f(t, c):
            s = s0 + t
            g = lax.div(s, NCH)
            for hs, hh in [(a, c) for a in range(HS) for c in range(G)]:
                off = pl.multiple_of(lax.rem(s, NCH) * CH + hs * (W // HS), CH)
                h = g * G + hh
                for b in range(B):
                    i = h * B + b
                    for pr, (src, dst) in enumerate(((k_hbm, kv.at[0]), (v_hbm, kv.at[1]))):
                        pltpu.make_async_copy(src.at[b, h, pl.ds(SK - W + off, CH), :],
                                              dst.at[i, pl.ds(off, CH), :], sem.at[SR + lax.rem(g, RING)]).start(priority=pr)
            return c
        lax.fori_loop(0, n, f, 0)

    def wait_all(ref, sem):
        pltpu.make_async_copy(ref, ref, sem).wait()

    c_x = pltpu.make_async_copy(x_hbm, x_v, sem.at[SQ])
    c_b1 = pltpu.make_async_copy(b1_hbm, b1_v, sem.at[SQ])
    c_b2 = pltpu.make_async_copy(b2_hbm, b2_v, sem.at[SQ])

    c_x.start()
    c_b1.start()
    c_b2.start()
    w_steps(wq_hbm, wq_v, sem.at[0], 0, WST // 2)
    c_x.wait()
    c_b1.wait()
    c_b2.wait()
    xs = x_v[...].astype(F32)
    row = lax.broadcasted_iota(jnp.int32, (8, D), 0)
    x8 = jnp.where(row % 2 == 0, xs[0:1, :], xs[1:2, :])
    m = jnp.mean(x8, axis=-1, keepdims=True)
    xc = x8 - m
    var = jnp.mean(xc * xc, axis=-1, keepdims=True)
    xn = (xc / jnp.sqrt(var + 1e-5)).astype(BF16)
    b1f_v[...] = b1_v[...].astype(F32)
    y0 = jnp.broadcast_to(b2_v[...].astype(F32).reshape(1, D), (8, D))
    w_steps(wq_hbm, wq_v, sem.at[0], WST // 2, WST - WST // 2)

    w_steps(w1_hbm, w1_v, sem.at[1], 0, WPRE)
    nw = (WST - WPRE) // WS
    wait_all(wq_v, sem.at[0])

    def qproj(j, c):
        c0 = pl.multiple_of(j * 512, 512)
        q_v[:, pl.ds(c0, 512)] = jnp.dot(xn, wq_v[:, pl.ds(c0, 512)], preferred_element_type=F32)

        @pl.when(j < nw)
        def _():
            w_steps(w1_hbm, w1_v, sem.at[1], WPRE + WS * j, WS)
        return c
    lax.fori_loop(0, HQ * DH // 512, qproj, 0)

    w_steps(w2t_hbm, w2t_v, sem.at[2], 0, WPRE)
    wait_all(w1_v, sem.at[1])

    def hproj(j, c):
        c0 = pl.multiple_of(j * 512, 512)
        hj = jnp.dot(xn, w1_v[:, pl.ds(c0, 512)], preferred_element_type=F32)
        bb = b1f_v[pl.ds(j * 4, 4), :]
        hj = hj + jnp.concatenate([bb[t:t + 1, :] for t in range(4)], axis=1)
        h_v[:, pl.ds(c0, 512)] = jax.nn.gelu(hj, approximate=True)

        @pl.when(j < nw)
        def _():
            w_steps(w2t_hbm, w2t_v, sem.at[2], WPRE + WS * j, WS)
        return c
    lax.fori_loop(0, F // 512, hproj, 0)

    ks = (NCH - PRE) // 8
    kv_steps(0, NCH - 8 * ks)
    wait_all(w2t_v, sem.at[2])

    def yproj(j, y):
        c0 = pl.multiple_of(j * 512, 512)
        y = y + lax.dot_general(h_v[:, pl.ds(c0, 512)].astype(BF16), w2t_v[:, pl.ds(c0, 512)], NT,
                                preferred_element_type=F32)

        @pl.when(j < 8)
        def _():
            kv_steps(NCH - 8 * ks + ks * j, ks)
        return y
    y = lax.fori_loop(0, F // 512, yproj, y0)
    gate = y * jax.nn.sigmoid(y)
    kv_steps(NCH, LA * (SPP // NSL))

    scale = DH ** -0.5
    r8 = lax.broadcasted_iota(jnp.int32, (8, DH), 0)
    RL = 512
    qw = HQ * DH // NQ
    qcs = max(1, CS // NQ) if qw * RW * 2 > 32768 else 1
    SPS = SPP // NSL

    def issue(i, part):
        slot = NSL * (i + PG) + part + LA

        @pl.when(slot < NSL * NP)
        def _():
            kv_steps(slot * SPS, SPS)

        @pl.when(slot >= NSL * NP)
        def _():
            t = slot - NSL * NP

            @pl.when(t < RL // 128)
            def _():
                w_steps(wot_hbm, wot_v, sem.at[t], 0, OS, r0=t * 128, per=OS)

            @pl.when(t == RL // 128)
            def _():
                for qi in range(NQ):
                    cw = qw // qcs
                    n = 0
                    for cc in range(qcs):
                        for r in range(RL, D, RW):
                            sl = (pl.ds(r, RW), pl.ds(qi * qw + cc * cw, cw))
                            pltpu.make_async_copy(wot_hbm.at[sl], wot_v.at[sl], sem.at[SQ + qi]).start(priority=n % 2)
                            n += 1

    def pair(i, c):
        h = lax.div(i, B)
        b = lax.rem(i, B)
        c0 = pl.multiple_of(h * 256, 256)
        hw = W // (NSL // 2)
        qh = jnp.where(r8 < 2, q_v[:, pl.ds(c0, 128)], q_v[:, pl.ds(c0 + 128, 128)]).astype(BF16)
        for j in range(NSL // 2):
            issue(i, j)
            if j == 0:
                @pl.when(lax.rem(i, PG) == 0)
                def _():
                    wait_all(kv.at[:, pl.ds(i, PG)], sem.at[SR + lax.rem(lax.div(i, PG), RING)])
            s_v[:, j * hw:(j + 1) * hw] = lax.dot_general(qh, kv[0, i, j * hw:(j + 1) * hw, :], NT,
                                                          preferred_element_type=F32) * scale
        s = s_v[...]
        mx = jnp.max(s, axis=-1, keepdims=True)
        p = jnp.exp(s - mx)
        l = jnp.sum(p, axis=-1, keepdims=True)
        s_v[...] = p
        o = jnp.zeros((8, DH), F32)
        for j in range(NSL // 2):
            issue(i, NSL // 2 + j)
            o = o + jnp.dot(s_v[:, j * hw:(j + 1) * hw].astype(BF16), kv[1, i, j * hw:(j + 1) * hw, :],
                            preferred_element_type=F32)
        o = o / l
        r0 = pl.multiple_of(b * 8, 8)
        oc_v[pl.ds(r0, 8), pl.ds(c0, 128)] = jnp.where(r8 == b, o, 0.0)
        oc_v[pl.ds(r0, 8), pl.ds(c0 + 128, 128)] = jnp.where(r8 == 2 + b, o, 0.0)
        return c
    lax.fori_loop(0, NP, pair, 0)

    oc = oc_v[...].astype(BF16)

    def oproj(t, c):
        r0 = pl.multiple_of(t * 128, 128)
        wait_all(wot_v.at[pl.ds(r0, 128), :], sem.at[t])
        oq = lax.dot_general(oc, wot_v[pl.ds(r0, 128), :], NT, preferred_element_type=F32)
        s_v[:, pl.ds(r0, 128)] = oq[0:8, :] + oq[8:16, :]
        return c
    lax.fori_loop(0, RL // 128, oproj, 0)
    sa = s_v[:, 0:RL]
    o_ref[:, 0:RL] = (xs[:, 0:RL] + (sa[0:2, :] + sa[2:4, :]) * gate[0:2, 0:RL]).astype(o_ref.dtype)
    acc = jnp.zeros((16, D - RL), F32)
    for qi in range(NQ):
        sl = (pl.ds(RL, D - RL), pl.ds(qi * qw, qw))
        wait_all(wot_v.at[sl], sem.at[SQ + qi])
        acc = acc + lax.dot_general(oc[:, qi * qw:(qi + 1) * qw], wot_v[sl], NT, preferred_element_type=F32)
    sb = acc[0:8, :] + acc[8:16, :]
    o_ref[:, RL:D] = (xs[:, RL:D] + (sb[0:2, :] + sb[2:4, :]) * gate[0:2, RL:D]).astype(o_ref.dtype)


@jax.jit
def pallas_recurrent_scan__sliding_block_cached__dense_activation_gelu__decode_kernel(
    A_x, A_k_cache, A_v_cache, A_wq, A_wo, B_x, B_w1, B_b1, B_w2, B_b2):
    CH = 64
    G = 1
    CS = 2
    NQ = 2
    PRE = 16
    LA = 2
    WPRE = 6
    NSL = 2
    NS = 4
    HS = 2
    B, Sq, D = A_x.shape
    _, HKV, SK, _ = A_k_cache.shape
    F = B_w1.shape[1]
    W = min(4096, max(256, SK // 4))
    bf = jnp.bfloat16
    anyspec = pl.BlockSpec(memory_space=pl.ANY)
    out = pl.pallas_call(
        functools.partial(_kernel, W=W, CH=CH, G=G, CS=CS, NQ=NQ, PRE=PRE, LA=LA, WPRE=WPRE, NSL=NSL, NS=NS, HS=HS),
        out_shape=jax.ShapeDtypeStruct((B, D), A_x.dtype),
        in_specs=[anyspec] * 9,
        out_specs=pl.BlockSpec(memory_space=pltpu.VMEM),
        scratch_shapes=[
            pltpu.VMEM((B, D), bf), pltpu.VMEM((F // 128, 128), bf), pltpu.VMEM((D,), bf),
            pltpu.VMEM((D, HQ * DH), bf), pltpu.VMEM((D, HQ * DH), bf),
            pltpu.VMEM((D, F), bf), pltpu.VMEM((D, F), bf),
            pltpu.VMEM((2, B * HKV, W, DH), bf),
            pltpu.VMEM((F // 128, 128), F32), pltpu.VMEM((8, HQ * DH), F32), pltpu.VMEM((8, F), F32),
            pltpu.VMEM((8, W), F32), pltpu.VMEM((16, HQ * DH), F32),
            pltpu.SemaphoreType.DMA((7 + NQ,)),
        ],
        compiler_params=pltpu.CompilerParams(vmem_limit_bytes=110 * 1024 * 1024, disable_bounds_checks=True),
    )(A_x.reshape(B, D), A_k_cache, A_v_cache, A_wq, A_wo.T, B_w1, B_b1.reshape(F // 128, 128), B_w2.T, B_b2)
    return out.reshape(B, Sq, D)
```

```python
import jax
import jax.numpy as jnp
from jax import lax
import jax.experimental.pallas as pl
import jax.experimental.pallas.tpu as pltpu

F32 = jnp.float32
BF16 = jnp.bfloat16
NT = (((1,), (1,)), ((), ()))

HQ, DH = 32, 128
KV_ROWS = 64
KV_SPLIT = 2
W_ROWS = 8
W_COLS = 2
W_STREAMS = 4
W_AHEAD = 6
KV_AHEAD = 16
LOOKAHEAD = 2
COLS = 512
RING = 3
N_WSEM = 4


def _wait_all(ref, sem):
    pltpu.make_async_copy(ref, ref, sem).wait()


def _kernel(x_hbm, k_hbm, v_hbm, wq_hbm, wot_hbm, w1_hbm, b1_hbm, w2t_hbm, b2_hbm,
            o_ref,
            x_v, b1_v, b2_v, wq_v, wot_v, w1_v, w2t_v, kv_v,
            b1f_v, q_v, h_v, s_v, oc_v, tail_sem):
    B, HKV, SK, _ = k_hbm.shape
    W = kv_v.shape[2]
    D = x_v.shape[1]
    F = w1_v.shape[1]
    n_pairs = B * HKV
    kv_nsteps = W // KV_ROWS // KV_SPLIT
    slot_steps = kv_nsteps // (2 * B)
    w_nsteps = D // W_ROWS // W_STREAMS
    d_main = D // 128 * 128
    n_groups = d_main // 128
    assert B == 2 and HQ == 2 * HKV and n_groups <= N_WSEM
    assert n_groups < 2 * B + LOOKAHEAD <= 2 * B * (RING - 1)

    def main(sem):
        small_sem = sem.at[N_WSEM + RING]

        def weight_steps(src, dst, wsem, t0, n, r0=0, rows=D):
            per = rows // W_ROWS // W_STREAMS
            cw = src.shape[1] // W_COLS

            def step(t, carry):
                for c in range(W_COLS):
                    for st in range(W_STREAMS):
                        r = pl.multiple_of(r0 + (st * per + t0 + t) * W_ROWS, W_ROWS)
                        sl = (pl.ds(r, W_ROWS), pl.ds(c * cw, cw))
                        pltpu.make_async_copy(src.at[sl], dst.at[sl], wsem).start(priority=st % 2)
                return carry
            lax.fori_loop(0, n, step, 0)

        def kv_steps(s0, n):
            def step(t, carry):
                h = lax.div(s0 + t, kv_nsteps)
                base = lax.rem(s0 + t, kv_nsteps) * KV_ROWS
                hsem = sem.at[N_WSEM + lax.rem(h, RING)]
                for part in range(KV_SPLIT):
                    off = pl.multiple_of(base + part * (W // KV_SPLIT), KV_ROWS)
                    for j, src in enumerate((k_hbm, v_hbm)):
                        for b in range(B):
                            pltpu.make_async_copy(
                                src.at[b, h, pl.ds(SK - W + off, KV_ROWS), :],
                                kv_v.at[j, h * B + b, pl.ds(off, KV_ROWS), :],
                                hsem).start(priority=b)
                return carry
            lax.fori_loop(0, n, step, 0)

        small = [pltpu.make_async_copy(s, d, small_sem)
                 for s, d in ((x_hbm, x_v), (b1_hbm, b1_v), (b2_hbm, b2_v))]
        for c in small:
            c.start()
        weight_steps(wq_hbm, wq_v, sem.at[0], 0, w_nsteps // 2)
        for c in small:
            c.wait()
        xs = x_v[...].astype(F32)
        row = lax.broadcasted_iota(jnp.int32, (8, D), 0)
        x8 = jnp.where(row % 2 == 0, xs[0:1, :], xs[1:2, :])
        xc = x8 - jnp.mean(x8, axis=-1, keepdims=True)
        var = jnp.mean(xc * xc, axis=-1, keepdims=True)
        xn = (xc / jnp.sqrt(var + 1e-5)).astype(BF16)
        b1f_v[...] = b1_v[...].astype(F32)
        y0 = jnp.broadcast_to(b2_v[...].astype(F32).reshape(1, D), (8, D))
        weight_steps(wq_hbm, wq_v, sem.at[0], w_nsteps // 2, w_nsteps - w_nsteps // 2)

        def rest_of(src, dst, wsem, j):
            @pl.when(W_AHEAD + 2 * j < w_nsteps)
            def _():
                weight_steps(src, dst, wsem, W_AHEAD + 2 * j, 2)

        weight_steps(w1_hbm, w1_v, sem.at[1], 0, W_AHEAD)
        _wait_all(wq_v, sem.at[0])

        def q_proj(j, carry):
            cols = pl.ds(pl.multiple_of(j * COLS, COLS), COLS)
            q_v[:, cols] = jnp.dot(xn, wq_v[:, cols], preferred_element_type=F32)
            rest_of(w1_hbm, w1_v, sem.at[1], j)
            return carry
        lax.fori_loop(0, HQ * DH // COLS, q_proj, 0)

        weight_steps(w2t_hbm, w2t_v, sem.at[2], 0, W_AHEAD)
        _wait_all(w1_v, sem.at[1])

        def hidden(j, carry):
            cols = pl.ds(pl.multiple_of(j * COLS, COLS), COLS)
            bias = b1f_v[pl.ds(j * (COLS // 128), COLS // 128), :]
            bias = jnp.concatenate([bias[t:t + 1, :] for t in range(COLS // 128)], axis=1)
            pre = jnp.dot(xn, w1_v[:, cols], preferred_element_type=F32) + bias
            h_v[:, cols] = jax.nn.gelu(pre, approximate=True)
            rest_of(w2t_hbm, w2t_v, sem.at[2], j)
            return carry
        lax.fori_loop(0, F // COLS, hidden, 0)

        kv_steps(0, KV_AHEAD)
        _wait_all(w2t_v, sem.at[2])

        def down_proj(j, y):
            cols = pl.ds(pl.multiple_of(j * COLS, COLS), COLS)
            y = y + lax.dot_general(h_v[:, cols].astype(BF16), w2t_v[:, cols], NT,
                                    preferred_element_type=F32)

            @pl.when(KV_AHEAD + 2 * j < kv_nsteps)
            def _():
                kv_steps(KV_AHEAD + 2 * j, 2)
            return y
        y = lax.fori_loop(0, F // COLS, down_proj, y0)
        gate = y * jax.nn.sigmoid(y)
        kv_steps(kv_nsteps, LOOKAHEAD * slot_steps)

        def issue(i, half):
            slot = 2 * (i + B) + half + LOOKAHEAD
            t = slot - 2 * n_pairs

            @pl.when(t < 0)
            def _():
                kv_steps(slot * slot_steps, slot_steps)

            @pl.when(t >= 0)
            def _():
                @pl.when(t < n_groups)
                def _():
                    weight_steps(wot_hbm, wot_v, sem.at[t], 0, 128 // W_ROWS // W_STREAMS,
                                 r0=t * 128, rows=128)

                @pl.when(t == n_groups)
                def _():
                    for n, r in enumerate(range(d_main, D, W_ROWS)):
                        rows = pl.ds(r, W_ROWS)
                        pltpu.make_async_copy(wot_hbm.at[rows, :], wot_v.at[rows, :],
                                              tail_sem).start(priority=n % 2)

        r8 = lax.broadcasted_iota(jnp.int32, (8, DH), 0)

        def attend(i, carry):
            h, b = lax.div(i, B), lax.rem(i, B)
            c0 = pl.multiple_of(h * 2 * DH, 2 * DH)
            q = jnp.where(r8 < 2, q_v[:, pl.ds(c0, DH)], q_v[:, pl.ds(c0 + DH, DH)]).astype(BF16)
            issue(i, 0)

            @pl.when(b == 0)
            def _():
                _wait_all(kv_v.at[:, pl.ds(i, B)], sem.at[N_WSEM + lax.rem(h, RING)])

            s = lax.dot_general(q, kv_v[0, i], NT, preferred_element_type=F32) * (DH ** -0.5)
            p = jnp.exp(s - jnp.max(s, axis=-1, keepdims=True))
            denom = jnp.sum(p, axis=-1, keepdims=True)
            s_v[...] = p
            issue(i, 1)
            o = jnp.dot(s_v[...].astype(BF16), kv_v[1, i], preferred_element_type=F32) / denom
            rows = pl.ds(pl.multiple_of(b * 8, 8), 8)
            oc_v[rows, pl.ds(c0, DH)] = jnp.where(r8 == b, o, 0.0)
            oc_v[rows, pl.ds(c0 + DH, DH)] = jnp.where(r8 == 2 + b, o, 0.0)
            return carry
        lax.fori_loop(0, n_pairs, attend, 0)

        oc = (oc_v[0:8, :] + oc_v[8:16, :]).astype(BF16)

        def out_proj(t, carry):
            rows = pl.ds(pl.multiple_of(t * 128, 128), 128)
            _wait_all(wot_v.at[rows, :], sem.at[t])
            s_v[:, rows] = lax.dot_general(oc, wot_v[rows, :], NT, preferred_element_type=F32)
            return carry
        lax.fori_loop(0, n_groups, out_proj, 0)
        s = s_v[:, 0:d_main]
        o_ref[:, 0:d_main] = (
            xs[:, 0:d_main] + (s[0:2, :] + s[2:4, :]) * gate[0:2, 0:d_main]).astype(o_ref.dtype)
        return xs, gate, oc

    xs, gate, oc = pl.run_scoped(main, pltpu.SemaphoreType.DMA((N_WSEM + RING + 1,)))

    _wait_all(wot_v.at[d_main:D, :], tail_sem)
    s = lax.dot_general(oc, wot_v[d_main:D, :], NT, preferred_element_type=F32)
    o_ref[:, d_main:D] = (
        xs[:, d_main:D] + (s[0:2, :] + s[2:4, :]) * gate[0:2, d_main:D]).astype(o_ref.dtype)


@jax.jit
def pallas_recurrent_scan__sliding_block_cached__dense_activation_gelu__decode_kernel(
    A_x: jax.Array,
    A_k_cache: jax.Array,
    A_v_cache: jax.Array,
    A_wq: jax.Array,
    A_wo: jax.Array,
    B_x: jax.Array,
    B_w1: jax.Array,
    B_b1: jax.Array,
    B_w2: jax.Array,
    B_b2: jax.Array,
):
    del B_x
    B, Sq, D = A_x.shape
    _, HKV, SK, _ = A_k_cache.shape
    F = B_w1.shape[1]
    W = min(4096, max(256, SK // 4))

    out = pl.pallas_call(
        _kernel,
        out_shape=jax.ShapeDtypeStruct((B * Sq, D), A_x.dtype),
        in_specs=[pl.BlockSpec(memory_space=pl.ANY)] * 9,
        out_specs=pl.BlockSpec(memory_space=pltpu.VMEM),
        scratch_shapes=[
            pltpu.VMEM((B * Sq, D), BF16),
            pltpu.VMEM((F // 128, 128), BF16),
            pltpu.VMEM((D,), BF16),
            pltpu.VMEM((D, HQ * DH), BF16),
            pltpu.VMEM((D, HQ * DH), BF16),
            pltpu.VMEM((D, F), BF16),
            pltpu.VMEM((D, F), BF16),
            pltpu.VMEM((2, B * HKV, W, DH), BF16),
            pltpu.VMEM((F // 128, 128), F32),
            pltpu.VMEM((8, HQ * DH), F32),
            pltpu.VMEM((8, F), F32),
            pltpu.VMEM((8, W), F32),
            pltpu.VMEM((16, HQ * DH), F32),
            pltpu.SemaphoreType.DMA(()),
        ],
        compiler_params=pltpu.CompilerParams(
            vmem_limit_bytes=110 * 1024 * 1024,
            disable_bounds_checks=True,
        ),
    )(A_x.reshape(B * Sq, D), A_k_cache, A_v_cache, A_wq, A_wo.T, B_w1,
      B_b1.reshape(F // 128, 128), B_w2.T, B_b2)
    return out.reshape(B, Sq, D)
```
